```python
import os as _os
_os.environ.setdefault('JAX_PLATFORMS', 'cpu')
import jax
import jax.numpy as jnp

def _softmax(x, axis=-1):
    return jax.nn.softmax(x, axis=axis)

def _gelu(x):
    return jax.nn.gelu(x, approximate=True)

def _silu(x):
    return jax.nn.silu(x)

def _sigmoid(x):
    return jax.nn.sigmoid(x)

def _layernorm(x, axis=-1, eps=1e-05):
    m = jnp.mean(x, axis=axis, keepdims=True)
    v = jnp.var(x, axis=axis, keepdims=True)
    return (x - m) / jnp.sqrt(v + eps)

def _scatter_add(tgt, idx, src, axis=0):
    return tgt.at[idx].add(src)

def _segment_sum(src, seg, n):
    return jax.ops.segment_sum(src, seg, n)

class _Rng:

    def __init__(self, key):
        self._k = key

    def _next(self):
        self._k, sub = jax.random.split(self._k)
        return sub

    def normal(self, shape):
        return jax.random.normal(self._next(), shape, dtype=jnp.bfloat16)

    def randint(self, lo, hi, shape):
        return jax.random.randint(self._next(), shape, lo, hi, dtype=jnp.int32)

    def uniform(self, shape, lo=0.0, hi=1.0):
        return jax.random.uniform(self._next(), shape, jnp.bfloat16, lo, hi)

    def permutation(self, n):
        return jax.random.permutation(self._next(), n)
kernel_name = 'adaLN_cond__sliding_block__dense_activation_silu__prompt'

def setup_inputs():
    _rng = _Rng(jax.random.key(int.from_bytes(__import__("os").urandom(4), "little")))
    _w = lambda a: (lambda t: t.astype(jnp.bfloat16) if jnp.issubdtype(t.dtype, jnp.floating) else t)(jnp.asarray(a))

    def _A_setup():
        B, S, D = (1, 2048, 512)
        return {'x': _w((lambda *s: _rng.normal(s) * 0.05)(B, S, D)), 'wqkv': _w((lambda *s: _rng.normal(s) * 0.05)(D, 3 * D)), 'wo': _w((lambda *s: _rng.normal(s) * 0.05)(D, D))}
    _A_in = _A_setup()

    def _B_setup():
        B, S, D, F = (1, 2048, 512, 1792)
        return {'x': _w((lambda *s: _rng.normal(s) * 0.05)(B, S, D)), 'w1': _w((lambda *s: _rng.normal(s) * 0.8)(D, F) * D ** (-0.5)), 'w2': _w((lambda *s: _rng.normal(s) * 0.8)(F, D) * F ** (-0.5))}
    _B_in = _B_setup()
    return {'A_x': _A_in['x'], 'A_wqkv': _A_in['wqkv'], 'A_wo': _A_in['wo'], 'B_x': _B_in['x'], 'B_w1': _B_in['w1'], 'B_w2': _B_in['w2'], 'c': _w((lambda *s: _rng.normal(s) * 0.05)(1, 512) * 8.0), 'w_mod': _w((lambda *s: _rng.normal(s) * 0.05)(512, 6 * 512) * 512 ** (-0.5) * 8.0)}

def reference(A_x, A_wqkv, A_wo, B_x, B_w1, B_w2, c, w_mod):

    def _A_ref(x, wqkv, wo):
        B, S, D = x.shape
        H = 32
        Dh = D // H
        W = 256
        qkv = (lambda x, *d: x.transpose(*d))((x @ wqkv).reshape(B, S, 3, H, Dh), 2, 0, 3, 1, 4)
        q, k, v = (qkv[0], qkv[1], qkv[2])
        scores = jnp.einsum('bhqd,bhkd->bhqk', q, k) * Dh ** (-0.5)
        idx = jnp.arange(S)
        mask = (idx[:, None] - idx[None, :] >= 0) & (idx[:, None] - idx[None, :] < W)
        scores = jnp.where(mask[None, None], scores, -1000000000.0)
        p = _softmax(scores, axis=-1)
        o = jnp.einsum('bhqk,bhkd->bhqd', p, v)
        return (lambda x, *d: x.transpose(*d))(o, 0, 2, 1, 3).reshape(B, S, D) @ wo

    def _B_ref(x, w1, w2):
        h = jnp.einsum('bsd,df->bsf', x, w1)
        h = _silu(h)
        out = jnp.einsum('bsf,fd->bsd', h, w2)
        return out
    x = A_x
    mod = (_silu(c) @ w_mod).reshape(c.shape[0], 6, 1, -1)
    sa, ca, ga, sb, cb, gb = (mod[:, 0].copy(), mod[:, 1].copy(), mod[:, 2].copy(), mod[:, 3].copy(), mod[:, 4].copy(), mod[:, 5].copy())
    h = _layernorm(x, axis=-1) * (1 + ca) + sa
    x = x + ga * _A_ref(h, A_wqkv, A_wo)
    h = _layernorm(x, axis=-1) * (1 + cb) + sb
    x = x + gb * _B_ref(h, B_w1, B_w2)
    return x
```

```python
import functools
import jax
import jax.numpy as jnp
from jax import lax
import jax.experimental.pallas as pl
import jax.experimental.pallas.tpu as pltpu

F32 = jnp.float32
BF16 = jnp.bfloat16
U32 = jnp.uint32
D = 512
H = 32
DH = 16
W = 256
EPS = 1e-5
LOG2E = 1.4426950408889634
NEG = -1e30


def _ln(x):
    m = jnp.mean(x, axis=-1, keepdims=True)
    xc = x - m
    v = jnp.mean(xc * xc, axis=-1, keepdims=True)
    return xc * lax.rsqrt(v + EPS)


def _nt(a, b):
    return lax.dot_general(a, b, (((1,), (1,)), ((), ())), preferred_element_type=F32)


def _nn(a, b):
    return jnp.dot(a, b, preferred_element_type=F32)


def _packi(x):
    r, c = x.shape
    x4 = x.reshape(r // 16, 2, 8, c)
    p = pltpu.pack_elementwise([x4[:, 0], x4[:, 1]], packed_dtype=BF16)
    return p.reshape(r // 2, c)


def _packc(x):
    return pltpu.bitcast(x.astype(BF16), U32)


def _asbf(x):
    return pltpu.bitcast(x, BF16)


def _qk(G, qT, kwin, slab_head0, nvalid_blocks):
    QW = 128 // G
    NC = 2 * G + 1
    first_valid_row = (3 - nvalid_blocks) * 128
    lane8 = lax.broadcasted_iota(jnp.int32, (8, 128), 1)
    grp8 = lane8 // QW
    rq = []
    for hh in range(G):
        r = qT[hh] if hh == 0 else pltpu.roll(qT[hh], QW * hh, 1)
        rq.append(r)
    zero8 = jnp.zeros((8, 128), U32)
    S = []
    for j in range(G):
        blocks = []
        for b in range(8):
            hh = b - slab_head0
            if 0 <= hh < G:
                blocks.append(jnp.where(grp8 == (j + hh) % G, rq[hh], zero8))
            else:
                blocks.append(zero8)
        wj = _asbf(jnp.concatenate(blocks, axis=0))
        c0 = max(0, first_valid_row // QW - j)
        S.append(_nn(kwin(QW * (j + c0), QW * (NC - c0)), wj))
    return S


def _barrel(G, A, shape, dtype):
    QW = 128 // G
    lane = lax.broadcasted_iota(jnp.int32, shape, 1) // QW
    zero = jnp.zeros(shape, dtype)
    cur = list(A)
    bit = 1
    while bit < G:
        sel = (lane & bit) != 0
        nxt = []
        for j in range(G):
            a, b = cur[(j + bit) % G], cur[j]
            if a is None and b is None:
                nxt.append(None)
            else:
                nxt.append(jnp.where(sel, zero if a is None else a, zero if b is None else b))
        cur = nxt
        bit *= 2
    return [zero if c is None else c for c in cur]


def _premax(G, S, nvalid_blocks):
    QW = 128 // G
    NC = 2 * G + 1
    first_valid_row = (3 - nvalid_blocks) * 128
    row = lax.broadcasted_iota(jnp.int32, (QW, 128), 0)
    ql = lax.broadcasted_iota(jnp.int32, (QW, 128), 1) % QW
    far_valid = row > ql
    res = []
    for j in range(G):
        s = S[j]
        c0 = max(0, first_valid_row // QW - j)
        last = s[(NC - 1 - c0) * QW:]
        ch = [None] * NC
        if c0 == 0:
            merged = jnp.where(far_valid, s[:QW], last)
        else:
            merged = jnp.where(far_valid, NEG, last)
        for c in range(max(c0, 1), NC - 1):
            ch[c] = s[(c - c0) * QW:(c - c0 + 1) * QW]
        ch[NC - 1] = merged
        m = None
        for c in range(1, NC):
            if ch[c] is not None:
                m = ch[c] if m is None else jnp.maximum(m, ch[c])
        m = jnp.max(m, axis=0, keepdims=True)
        res.append((ch, m, c0))
    return res


def _softmax_pv_gen(G, SM, nvalid_blocks, vts, res, mxu_sum):
    QW = 128 // G
    NC = 2 * G + 1
    row = lax.broadcasted_iota(jnp.int32, (QW, 128), 0)
    ql = lax.broadcasted_iota(jnp.int32, (QW, 128), 1) % QW
    far_valid = row > ql
    ones = jnp.full((8, 128), 0x3F803F80, U32)
    pm_cache = {}
    lsum = [None] * G

    def addsum(j, p):
        if mxu_sum:
            return
        s = p[0:8]
        for r in range(8, QW, 8):
            s = s + p[r:r + 8]
        lsum[j] = s if lsum[j] is None else lsum[j] + s

    def pchunk(j, c):
        ch, m, c0 = SM[j]
        if c < 0 or c >= NC or c < c0:
            return None
        if c == 0 or c == NC - 1:
            if j not in pm_cache:
                pm = jnp.exp2(ch[NC - 1] - m)
                addsum(j, pm)
                if c0 == 0:
                    pm_cache[j] = (_packi(jnp.where(far_valid, pm, 0.0)), _packi(jnp.where(far_valid, 0.0, pm)))
                else:
                    pm_cache[j] = (None, _packi(pm))
            return pm_cache[j][0 if c == 0 else 1]
        p = jnp.exp2(ch[c] - m)
        addsum(j, p)
        return _packi(p)

    acc = [None] * G
    for kt in range(3 - nvalid_blocks, 3):
        outs = [[] for _ in range(G)]
        for t in range(kt * G, (kt + 1) * G):
            A = [pchunk(j, t - j) for j in range(G)]
            Dj = _barrel(G, A, (QW // 2, 128), U32)
            for hh in range(G):
                outs[hh].append(Dj[(-hh) % G])
        for hh in range(G):
            pt = _asbf(jnp.concatenate(outs[hh], axis=0))
            if mxu_sum:
                vt = _asbf(jnp.concatenate([vts[hh][kt], ones], axis=0))
                o = _nn(vt, pt)[:24]
            else:
                o = _nn(_asbf(vts[hh][kt]), pt)
            acc[hh] = o if acc[hh] is None else acc[hh] + o
        if kt < 2:
            yield 'pv'
    if not mxu_sum:
        Ld = _barrel(G, lsum, (8, 128), F32)
    for hh in range(G):
        if mxu_sum:
            rl = pl.reciprocal(acc[hh][16:24], approx=True)
            o = acc[hh][:16] * jnp.concatenate([rl, rl], axis=0)
        else:
            l = jnp.sum(Ld[(-hh) % G], axis=0, keepdims=True)
            o = acc[hh] * pl.reciprocal(l, approx=True)
        if hh:
            o = pltpu.roll(o, 128 - QW * hh, 1)
        res.append(o)
    yield 'pv'


def make_kernel(TQ, G, S, F, LA, mxu_sum, dpat):
    NQ = TQ // 128
    NSTEP = S // TQ
    NF = F // 128

    def kernel(xa_ref, xb_ref, c_ref, wqkv_hbm, wo_hbm, w1_hbm, w2_hbm, wmod_hbm, o_ref,
               wqkv_ref, wo_ref, w1_ref, w2_ref, wmod_ref, sems,
               mod_s, wqvT_s, k_s, vT_s, o_s):
        i = pl.program_id(0)

        def cp(k):
            if k == 0:
                return pltpu.make_async_copy(wqkv_hbm, wqkv_ref, sems.at[0])
            if k == 1:
                return pltpu.make_async_copy(wmod_hbm.at[:, 0:2 * D], wmod_ref.at[:, 0:2 * D], sems.at[1])
            if k == 2:
                return pltpu.make_async_copy(wmod_hbm.at[:, 2 * D:6 * D], wmod_ref.at[:, 2 * D:6 * D], sems.at[2])
            if k == 3:
                return pltpu.make_async_copy(wo_hbm, wo_ref, sems.at[3])
            if k == 4:
                return pltpu.make_async_copy(w1_hbm, w1_ref, sems.at[4])
            return pltpu.make_async_copy(w2_hbm, w2_ref, sems.at[5])

        def modv(k):
            return mod_s[0:1, k * D:(k + 1) * D]

        def silu_c():
            c = c_ref[...].astype(F32)
            sc = (c * jax.nn.sigmoid(c)).astype(BF16)
            return jnp.broadcast_to(sc, (16, D))

        def A_gen(first):
            x = xa_ref[...].astype(F32)
            hf = _ln(x) * (1.0 + modv(1)) + modv(0)
            h = hf.astype(BF16)
            hp = _asbf(_packi(hf))
            yield 'ln'
            row0 = pl.multiple_of(i * (TQ // 2), TQ // 2)
            for cc in range(4):
                k_s[pl.ds(row0, TQ // 2), cc * 128:(cc + 1) * 128] = _packc(
                    _nn(h, wqkv_ref[:, D + cc * 128:D + (cc + 1) * 128]))
                yield 'k'
            qT = []
            for b in range(NQ):
                qT.append(_packc(_nt(_asbf(wqvT_s[0:D // 2, :]), h[b * 128:(b + 1) * 128]) * (DH ** -0.5 * LOG2E)))
                yield 'q'
            for b in range(NQ):
                vT_s[i * NQ + b] = _packc(_nt(_asbf(wqvT_s[D // 2:D, :]), hp[b * 128:(b + 1) * 128]))
                yield 'v'

            groups = [(b, h0) for b in range(NQ) for h0 in range(0, H, G)]

            def nvalid(b):
                return min(3, b + 1) if first else 3

            def qk(n):
                b, h0 = groups[n]
                slab = h0 // 8

                def kwin(start, size):
                    s2 = (b * 128 - 256 + start) // 2
                    if first:
                        return _asbf(k_s[s2:s2 + size // 2, slab * 128:(slab + 1) * 128])
                    st = pl.multiple_of(row0 + s2, 8)
                    return _asbf(k_s[pl.ds(st, size // 2), slab * 128:(slab + 1) * 128])
                qs = [qT[b][(h0 + hh) * 8:(h0 + hh + 1) * 8] for hh in range(G)]
                return _premax(G, _qk(G, qs, kwin, h0 % 8, nvalid(b)), nvalid(b))

            NG = len(groups)
            Sq = []
            for n in range(min(LA, NG)):
                Sq.append(qk(n))
                yield 'qk'
            oT = []
            for n in range(NG):
                if n + LA < NG:
                    Sq.append(qk(n + LA))
                    yield 'qk'
                b, h0 = groups[n]
                vts = []
                for hh in range(G):
                    hd = h0 + hh
                    vts.append([vT_s[i * NQ + b - 2 + t, hd * 8:(hd + 1) * 8, :]
                                if t >= 3 - nvalid(b) else None for t in range(3)])
                yield from _softmax_pv_gen(G, Sq[n], nvalid(b), vts, oT, mxu_sum)
                if h0 + G == H:
                    oTb = jnp.concatenate(oT[b * H:(b + 1) * H], axis=0).astype(BF16)
                    o_s[b * 64:(b + 1) * 64, :] = pltpu.bitcast(oTb.T, U32)

        def B_gen():
            o = _asbf(o_s[...])
            att = []
            for cc in range(4):
                att.append(_nn(o, wo_ref[:, cc * 128:(cc + 1) * 128]))
                yield 'wo'
            x1 = xb_ref[...].astype(F32) + modv(2) * jnp.concatenate(att, axis=1)
            h2 = (_ln(x1) * (0.5 * (1.0 + modv(4))) + 0.5 * modv(3)).astype(BF16)
            yield 'ln'
            act = []
            y = [None] * 4

            def w1round(r):
                a = _nn(h2, w1_ref[:, r * 128:(r + 1) * 128])
                act.append((a + a * jnp.tanh(a)).astype(BF16))

            def w2round(g, cs):
                lo, hi = g * 4, min(g * 4 + 4, NF)
                for cc in cs:
                    for r in range(lo, hi):
                        t = _nn(act[r], w2_ref[r * 128:(r + 1) * 128, cc * 128:(cc + 1) * 128])
                        y[cc] = t if y[cc] is None else y[cc] + t

            order = []
            w1l = [('1', r) for r in range(NF)]
            w2l = []
            for g in range((NF + 3) // 4):
                nk = min(4, NF - g * 4)
                per = 4 // nk
                for c0 in range(0, 4, per):
                    w2l.append(('2', g, tuple(range(c0, c0 + per))))
            done1 = 0
            while w1l or w2l:
                if w1l and (done1 < 5 or not w2l or done1 < min(NF, w2l[0][1] * 4 + 5)):
                    order.append(w1l.pop(0)); done1 += 1
                else:
                    order.append(w2l.pop(0))
                    if w1l:
                        order.append(w1l.pop(0)); done1 += 1
            for it in order:
                if it[0] == '1':
                    w1round(it[1])
                else:
                    w2round(it[1], it[2])
                yield 'd'
            o_ref[...] = (x1 + modv(5) * jnp.concatenate(y, axis=1)).astype(o_ref.dtype)

        def drain(g):
            for _ in g:
                pass

        @pl.when(i == 0)
        def _():
            cp(0).start()
            cp(1).start()
            cp(0).wait()
            wqvT_s[0:D // 2, :] = pltpu.bitcast(wqkv_ref[:, 0:D].T, U32)
            wqvT_s[D // 2:D, :] = pltpu.bitcast(wqkv_ref[:, 2 * D:3 * D].T, U32)
            cp(1).wait()
            for k in (3, 2, 4, 5):
                cp(k).start()
            mod_s[:, 0:2 * D] = _nn(silu_c(), wmod_ref[:, 0:2 * D])[:8]
            drain(A_gen(True))
            cp(2).wait()
            mod_s[:, 2 * D:6 * D] = _nn(silu_c(), wmod_ref[:, 2 * D:6 * D])[:8]
            for k in (3, 4, 5):
                cp(k).wait()

        @pl.when(jnp.logical_and(i > 0, i < NSTEP))
        def _():
            a = A_gen(False)
            b = B_gen()
            next(a)
            for _ in range(4):
                next(b)
            next(b)
            for _ in range(4 + 2 * NQ):
                next(a)
            npv = 0
            for tag in a:
                if tag == 'pv':
                    nd = dpat(npv)
                    npv += 1
                    for _ in range(nd):
                        next(b, None)
            drain(b)

        @pl.when(i == NSTEP)
        def _():
            drain(B_gen())

    return kernel


def run(A_x, A_wqkv, A_wo, B_x, B_w1, B_w2, c, w_mod, TQ=256, G=4, LA=2, mxu_sum=True, dp=0):
    B, S, _ = A_x.shape
    F = B_w1.shape[1]
    x = A_x.reshape(S, D)
    n = S // TQ
    if dp == 0:
        dpat = lambda k: 1 if k % 3 != 2 else 0
    elif dp == 1:
        dpat = lambda k: 1 if (k % 3 != 2 and k >= 6) else 0
    elif dp == 2:
        dpat = lambda k: (1 if k % 3 == 0 else 0) if k < 12 else (1 if k % 3 != 2 else 0)
    elif dp == 3:
        dpat = lambda k: 0
    anyspec = pl.BlockSpec(memory_space=pl.ANY)
    out = pl.pallas_call(
        make_kernel(TQ, G, S, F, LA, mxu_sum, dpat),
        grid=(n + 1,),
        in_specs=[pl.BlockSpec((TQ, D), lambda i: (jnp.minimum(i, n - 1), 0)),
                  pl.BlockSpec((TQ, D), lambda i: (jnp.maximum(i - 1, 0), 0)),
                  pl.BlockSpec((1, D), lambda i: (0, 0)),
                  anyspec, anyspec, anyspec, anyspec, anyspec],
        out_specs=pl.BlockSpec((TQ, D), lambda i: (jnp.maximum(i - 1, 0), 0)),
        out_shape=jax.ShapeDtypeStruct((S, D), A_x.dtype),
        scratch_shapes=[pltpu.VMEM(A_wqkv.shape, BF16), pltpu.VMEM(A_wo.shape, BF16),
                        pltpu.VMEM(B_w1.shape, BF16), pltpu.VMEM(B_w2.shape, BF16),
                        pltpu.VMEM(w_mod.shape, BF16), pltpu.SemaphoreType.DMA((6,)),
                        pltpu.VMEM((8, 6 * D), F32), pltpu.VMEM((D, D), U32),
                        pltpu.VMEM((S // 2, D), U32), pltpu.VMEM((S // 128, D // 2, 128), U32),
                        pltpu.VMEM((TQ // 2, D), U32)],
        compiler_params=pltpu.CompilerParams(dimension_semantics=("arbitrary",),
                                             vmem_limit_bytes=64 * 1024 * 1024),
        name="adaln_k4",
    )(x, x, c, A_wqkv, A_wo, B_w1, B_w2, w_mod)
    return out.reshape(B, S, D)


@jax.jit
def pallas_adaLN_cond__sliding_block__dense_activation_silu__prompt_kernel(A_x, A_wqkv, A_wo, B_x, B_w1, B_w2, c, w_mod):
    return run(A_x, A_wqkv, A_wo, B_x, B_w1, B_w2, c, w_mod)
```

```python
import functools
import jax
import jax.numpy as jnp
from jax import lax
import jax.experimental.pallas as pl
import jax.experimental.pallas.tpu as pltpu

F32 = jnp.float32
BF16 = jnp.bfloat16
U32 = jnp.uint32
D = 512
H = 32
DH = 16
W = 256
EPS = 1e-5
LOG2E = 1.4426950408889634
NEG = -1e30


def _ln(x):
    m = jnp.mean(x, axis=-1, keepdims=True)
    xc = x - m
    v = jnp.mean(xc * xc, axis=-1, keepdims=True)
    return xc * lax.rsqrt(v + EPS)


def _nt(a, b):
    return lax.dot_general(a, b, (((1,), (1,)), ((), ())), preferred_element_type=F32)


def _nn(a, b):
    return jnp.dot(a, b, preferred_element_type=F32)


def _packi(x):
    r, c = x.shape
    x4 = x.reshape(r // 16, 2, 8, c)
    p = pltpu.pack_elementwise([x4[:, 0], x4[:, 1]], packed_dtype=BF16)
    return p.reshape(r // 2, c)


def _packc(x):
    return pltpu.bitcast(x.astype(BF16), U32)


def _asbf(x):
    return pltpu.bitcast(x, BF16)


def _qk(G, qT, kwin, slab_head0, nvalid_blocks):
    QW = 128 // G
    NC = 2 * G + 1
    first_valid_row = (3 - nvalid_blocks) * 128
    lane8 = lax.broadcasted_iota(jnp.int32, (8, 128), 1)
    grp8 = lane8 // QW
    rq = []
    for hh in range(G):
        r = qT[hh] if hh == 0 else pltpu.roll(qT[hh], QW * hh, 1)
        rq.append(r)
    zero8 = jnp.zeros((8, 128), U32)
    S = []
    for j in range(G):
        blocks = []
        for b in range(8):
            hh = b - slab_head0
            if 0 <= hh < G:
                blocks.append(jnp.where(grp8 == (j + hh) % G, rq[hh], zero8))
            else:
                blocks.append(zero8)
        wj = _asbf(jnp.concatenate(blocks, axis=0))
        c0 = max(0, first_valid_row // QW - j)
        S.append(_nn(kwin(QW * (j + c0), QW * (NC - c0)), wj))
    return S


def _barrel(G, A, shape, dtype):
    QW = 128 // G
    lane = lax.broadcasted_iota(jnp.int32, shape, 1) // QW
    zero = jnp.zeros(shape, dtype)
    cur = list(A)
    bit = 1
    while bit < G:
        sel = (lane & bit) != 0
        nxt = []
        for j in range(G):
            a, b = cur[(j + bit) % G], cur[j]
            if a is None and b is None:
                nxt.append(None)
            else:
                nxt.append(jnp.where(sel, zero if a is None else a, zero if b is None else b))
        cur = nxt
        bit *= 2
    return [zero if c is None else c for c in cur]


def _premax(G, S, nvalid_blocks, s_ref):
    QW = 128 // G
    NC = 2 * G + 1
    first_valid_row = (3 - nvalid_blocks) * 128
    row = lax.broadcasted_iota(jnp.int32, (QW, 128), 0)
    ql = lax.broadcasted_iota(jnp.int32, (QW, 128), 1) % QW
    far_valid = row > ql
    for j in range(G):
        s = S[j]
        c0 = max(0, first_valid_row // QW - j)
        last = s[(NC - 1 - c0) * QW:]
        ch = [None] * NC
        if c0 == 0:
            merged = jnp.where(far_valid, s[:QW], last)
        else:
            merged = jnp.where(far_valid, NEG, last)
        for c in range(max(c0, 1), NC - 1):
            ch[c] = s[(c - c0) * QW:(c - c0 + 1) * QW]
        ch[NC - 1] = merged
        m = None
        for c in range(1, NC):
            if ch[c] is not None:
                s_ref[j, (c - 1) * QW:c * QW, :] = ch[c]
                for r in range(0, QW, 8):
                    m = ch[c][r:r + 8] if m is None else jnp.maximum(m, ch[c][r:r + 8])
        m = jnp.max(m, axis=0, keepdims=True)
        s_ref[j, 256:264, :] = jnp.broadcast_to(m, (8, 128))
    return None


def _softmax_pv_gen(G, s_ref, nvalid_blocks, vts, res, mxu_sum):
    QW = 128 // G
    NC = 2 * G + 1
    first_valid_row = (3 - nvalid_blocks) * 128
    row = lax.broadcasted_iota(jnp.int32, (QW, 128), 0)
    ql = lax.broadcasted_iota(jnp.int32, (QW, 128), 1) % QW
    far_valid = row > ql
    ones = jnp.full((8, 128), 0x3F803F80, U32)
    pm_cache = {}
    lsum = [None] * G
    lcur = [None] * G

    def addsum(j, p):
        if mxu_sum:
            return
        for r in range(QW - 16, -1, -16):
            pr = p[r:r + 8] + p[r + 8:r + 16]
            lcur[j] = pr if lcur[j] is None else lcur[j] + pr

    def pexp(j, c):
        m = s_ref[j, 256:264, :]
        s = s_ref[j, (c - 1) * QW:c * QW, :]
        p = jnp.exp2(s - jnp.concatenate([m] * (QW // 8), axis=0))
        addsum(j, p)
        return p

    def pchunk(j, c):
        c0 = max(0, first_valid_row // QW - j)
        if c < 0 or c >= NC or c < c0:
            return None
        if c == 0 or c == NC - 1:
            if j not in pm_cache:
                pm = pexp(j, NC - 1)
                if c0 == 0:
                    pm_cache[j] = (_packi(jnp.where(far_valid, pm, 0.0)), _packi(jnp.where(far_valid, 0.0, pm)))
                else:
                    pm_cache[j] = (None, _packi(pm))
            return pm_cache[j][0 if c == 0 else 1]
        return _packi(pexp(j, c))

    acc = [None] * G
    for kt in range(3 - nvalid_blocks, 3):
        outs = [[] for _ in range(G)]
        for t in range((kt + 1) * G - 1, kt * G - 1, -1):
            A = [pchunk(j, t - j) for j in range(G)]
            Dj = _barrel(G, A, (QW // 2, 128), U32)
            for hh in range(G):
                outs[hh].insert(0, Dj[(-hh) % G])
        for j in range(G):
            if lcur[j] is not None:
                lsum[j] = lcur[j] if lsum[j] is None else lsum[j] + lcur[j]
                lcur[j] = None
        for hh in range(G):
            pt = _asbf(jnp.concatenate(outs[hh], axis=0))
            if mxu_sum:
                vt = _asbf(jnp.concatenate([vts[hh][kt], ones], axis=0))
                o = _nn(vt, pt)[:24]
            else:
                o = _nn(_asbf(vts[hh][kt]), pt)
            acc[hh] = o if acc[hh] is None else o + acc[hh]
        if kt < 2:
            yield 'pv'
    if not mxu_sum:
        Ld = _barrel(G, lsum, (8, 128), F32)
    for hh in range(G):
        if mxu_sum:
            rl = pl.reciprocal(acc[hh][16:24], approx=True)
            o = acc[hh][:16] * jnp.concatenate([rl, rl], axis=0)
        else:
            l = jnp.sum(Ld[(-hh) % G], axis=0, keepdims=True)
            o = acc[hh] * pl.reciprocal(l, approx=True)
        if hh:
            o = pltpu.roll(o, 128 - QW * hh, 1)
        res.append(o)
    yield 'pv'


def make_kernel(TQ, G, S, F, LA, mxu_sum, dpat, w2wait):
    NQ = TQ // 128
    NSTEP = S // TQ
    NF = F // 128

    def kernel(x_hbm, c_hbm, wqkv_hbm, wo_hbm, w1_hbm, w2_hbm, wmod_hbm, o_ref,
               x_s, c_ref, wqkv_ref, wo_ref, w1_ref, w2_ref, wmod_ref, sems,
               mod_s, wqvT_s, k_s, vT_s, o_s, s_s):
        i = pl.program_id(0)

        def colcp(src, dst, lo, hi, k):
            return pltpu.make_async_copy(src.at[:, lo:hi], dst.at[:, lo:hi], sems.at[k])

        def cp(name):
            if name == 'c':
                return pltpu.make_async_copy(c_hbm, c_ref, sems.at[0])
            if name == 'mod1':
                return colcp(wmod_hbm, wmod_ref, 0, 2 * D, 1)
            if name == 'wk':
                return colcp(wqkv_hbm, wqkv_ref, D, 2 * D, 2)
            if name == 'wq':
                return colcp(wqkv_hbm, wqkv_ref, 0, D, 3)
            if name == 'wv':
                return colcp(wqkv_hbm, wqkv_ref, 2 * D, 3 * D, 4)
            if name == 'wo':
                return pltpu.make_async_copy(wo_hbm, wo_ref, sems.at[5])
            if name == 'mod2':
                return colcp(wmod_hbm, wmod_ref, 2 * D, 6 * D, 6)
            if name == 'w1':
                return pltpu.make_async_copy(w1_hbm, w1_ref, sems.at[7])
            if name == 'w2':
                return pltpu.make_async_copy(w2_hbm, w2_ref, sems.at[8])
            raise ValueError(name)

        def xcp(t, k):
            r = t * TQ if isinstance(t, int) else pl.multiple_of(t * TQ, TQ)
            return pltpu.make_async_copy(x_hbm.at[pl.ds(r, TQ), :], x_s.at[pl.ds(r, TQ), :], sems.at[k])

        def modv(k):
            return mod_s[0:1, k * D:(k + 1) * D]

        def silu_c():
            c = c_ref[...].astype(F32)
            sc = (c * jax.nn.sigmoid(c)).astype(BF16)
            return jnp.broadcast_to(sc, (16, D))

        def A_gen(first):
            x = x_s[pl.ds(pl.multiple_of(i * TQ, TQ), TQ), :].astype(F32)
            hf = _ln(x) * (1.0 + modv(1)) + modv(0)
            h = hf.astype(BF16)
            hp = _asbf(_packi(hf))
            yield 'ln'
            row0 = pl.multiple_of(i * (TQ // 2), TQ // 2)
            for cc in range(4):
                k_s[pl.ds(row0, TQ // 2), cc * 128:(cc + 1) * 128] = _packc(
                    _nn(h, wqkv_ref[:, D + cc * 128:D + (cc + 1) * 128]))
                yield 'k'
            qT = []
            for b in range(NQ):
                qT.append(_packc(_nt(_asbf(wqvT_s[0:D // 2, :]), h[b * 128:(b + 1) * 128]) * (DH ** -0.5 * LOG2E)))
                yield 'q'
            for b in range(NQ):
                vT_s[i * NQ + b] = _packc(_nt(_asbf(wqvT_s[D // 2:D, :]), hp[b * 128:(b + 1) * 128]))
                yield 'v'

            groups = [(b, h0) for b in range(NQ) for h0 in range(0, H, G)]

            def nvalid(b):
                return min(3, b + 1) if first else 3

            def qk(n):
                b, h0 = groups[n]
                slab = h0 // 8

                def kwin(start, size):
                    s2 = (b * 128 - 256 + start) // 2
                    if first:
                        return _asbf(k_s[s2:s2 + size // 2, slab * 128:(slab + 1) * 128])
                    st = pl.multiple_of(row0 + s2, 8)
                    return _asbf(k_s[pl.ds(st, size // 2), slab * 128:(slab + 1) * 128])
                qs = [qT[b][(h0 + hh) * 8:(h0 + hh + 1) * 8] for hh in range(G)]
                return _premax(G, _qk(G, qs, kwin, h0 % 8, nvalid(b)), nvalid(b), s_s.at[n])

            NG = len(groups)
            for n in range(min(LA, NG)):
                qk(n)
                yield 'qk'
            oT = []
            for n in range(NG):
                if n + LA < NG:
                    qk(n + LA)
                    yield 'qk'
                b, h0 = groups[n]
                vts = []
                for hh in range(G):
                    hd = h0 + hh
                    vts.append([vT_s[i * NQ + b - 2 + t, hd * 8:(hd + 1) * 8, :]
                                if t >= 3 - nvalid(b) else None for t in range(3)])
                yield from _softmax_pv_gen(G, s_s.at[n], nvalid(b), vts, oT, mxu_sum)
                if h0 + G == H:
                    oTb = jnp.concatenate(oT[b * H:(b + 1) * H], axis=0).astype(BF16)
                    o_s[b * 64:(b + 1) * 64, :] = pltpu.bitcast(oTb.T, U32)
                yield 'g'

        def B_gen(lead):
            o = _asbf(o_s[...])
            att = []
            for cc in range(4):
                att.append(_nn(o, wo_ref[:, cc * 128:(cc + 1) * 128]))
                yield 'wo'
            xb = x_s[pl.ds(pl.multiple_of((i - 1) * TQ, TQ), TQ), :].astype(F32)
            x1 = xb + modv(2) * jnp.concatenate(att, axis=1)
            h2 = (_ln(x1) * (0.5 * (1.0 + modv(4))) + 0.5 * modv(3)).astype(BF16)
            yield 'ln'
            act = []
            y = [None] * 4

            def w1round(r):
                a = _nn(h2, w1_ref[:, r * 128:(r + 1) * 128])
                act.append((a + a * jnp.tanh(a)).astype(BF16))

            def w2round(g, cs):
                lo, hi = g * 4, min(g * 4 + 4, NF)
                for cc in cs:
                    for r in range(lo, hi):
                        t = _nn(act[r], w2_ref[r * 128:(r + 1) * 128, cc * 128:(cc + 1) * 128])
                        y[cc] = t if y[cc] is None else t + y[cc]

            order = []
            w1l = [('1', r) for r in range(NF)]
            w2l = []
            for g in range((NF + 3) // 4):
                nk = min(4, NF - g * 4)
                per = 4 // nk
                for c0 in range(0, 4, per):
                    w2l.append(('2', g, tuple(range(c0, c0 + per))))
            done1 = 0
            while w1l or w2l:
                if w1l and (done1 < lead or not w2l or done1 < min(NF, w2l[0][1] * 4 + 5)):
                    order.append(w1l.pop(0)); done1 += 1
                else:
                    order.append(w2l.pop(0))
                    if w1l:
                        order.append(w1l.pop(0)); done1 += 1
            for it in order:
                if it[0] == '1':
                    w1round(it[1])
                else:
                    w2round(it[1], it[2])
                yield 'd'
            o_ref[...] = (x1 + modv(5) * jnp.concatenate(y, axis=1)).astype(o_ref.dtype)

        def drain(g):
            for _ in g:
                pass

        @pl.when(i == 0)
        def _():
            xcp(0, 9).start()
            for nm in ('c', 'mod1', 'wk', 'wq', 'wv'):
                cp(nm).start()
            xcp(1, 10).start()
            for nm in ('wo', 'mod2', 'w1', 'w2'):
                cp(nm).start()
            xcp(0, 9).wait()
            cp('c').wait()
            cp('mod1').wait()
            mod_s[:, 0:2 * D] = _nn(silu_c(), wmod_ref[:, 0:2 * D])[:8]
            a = A_gen(True)
            next(a)
            cp('wk').wait()
            for _ in range(4):
                next(a)
            cp('wq').wait()
            wqvT_s[0:D // 2, :] = pltpu.bitcast(wqkv_ref[:, 0:D].T, U32)
            for _ in range(NQ):
                next(a)
            cp('wv').wait()
            wqvT_s[D // 2:D, :] = pltpu.bitcast(wqkv_ref[:, 2 * D:3 * D].T, U32)
            drain(a)
            cp('mod2').wait()
            mod_s[:, 2 * D:6 * D] = _nn(silu_c(), wmod_ref[:, 2 * D:6 * D])[:8]
            cp('wo').wait()

        @pl.when(jnp.logical_and(i > 0, i < NSTEP))
        def _():
            xcp(i, 10).wait()

        @pl.when(jnp.logical_and(i > 0, i + 1 < NSTEP))
        def _():
            xcp(i + 1, 10).start()

        def steady(second):
            a = A_gen(False)
            b = B_gen(w2wait + 1 if second else 5)
            next(a)
            for _ in range(4):
                next(b)
            next(b)
            for _ in range(4 + 2 * NQ):
                next(a)
            if second:
                cp('w1').wait()
            npv = 0
            nd_tot = 0
            for tag in a:
                if tag == 'pv':
                    nd = dpat(npv)
                    npv += 1
                    for _ in range(nd):
                        next(b, None)
                        nd_tot += 1
                        if second and nd_tot == w2wait:
                            cp('w2').wait()
            drain(b)

        @pl.when(i == 1)
        def _():
            steady(True)

        @pl.when(jnp.logical_and(i > 1, i < NSTEP))
        def _():
            steady(False)

        @pl.when(i == NSTEP)
        def _():
            drain(B_gen(5))

    return kernel


def run(A_x, A_wqkv, A_wo, B_x, B_w1, B_w2, c, w_mod, TQ=256, G=4, LA=2, mxu_sum=False, dp=8, w2wait=5):
    B, S, _ = A_x.shape
    F = B_w1.shape[1]
    x = A_x.reshape(S, D)
    n = S // TQ
    if dp == 0:
        dpat = lambda k: 1 if k % 3 != 2 else 0
    elif dp == 4:
        dpat = lambda k: 1 if k % 3 == 1 else 0
    elif dp == 5:
        dpat = lambda k: (1 if k % 3 == 1 else 0) if k < 24 else (1 if k % 3 != 2 else 0)
    elif dp == 8:
        dpat = lambda k: (1 if k % 3 == 1 else 0) if k < 18 else (1 if k % 3 != 2 else 0)
    anyspec = pl.BlockSpec(memory_space=pl.ANY)
    out = pl.pallas_call(
        make_kernel(TQ, G, S, F, LA, mxu_sum, dpat, w2wait),
        grid=(n + 1,),
        in_specs=[anyspec] * 7,
        out_specs=pl.BlockSpec((TQ, D), lambda i: (jnp.maximum(i - 1, 0), 0)),
        out_shape=jax.ShapeDtypeStruct((S, D), A_x.dtype),
        scratch_shapes=[pltpu.VMEM((S, D), BF16), pltpu.VMEM((1, D), BF16),
                        pltpu.VMEM(A_wqkv.shape, BF16), pltpu.VMEM(A_wo.shape, BF16),
                        pltpu.VMEM(B_w1.shape, BF16), pltpu.VMEM(B_w2.shape, BF16),
                        pltpu.VMEM(w_mod.shape, BF16), pltpu.SemaphoreType.DMA((11,)),
                        pltpu.VMEM((8, 6 * D), F32), pltpu.VMEM((D, D), U32),
                        pltpu.VMEM((S // 2, D), U32), pltpu.VMEM((S // 128, D // 2, 128), U32),
                        pltpu.VMEM((TQ // 2, D), U32),
                        pltpu.VMEM((TQ // 128 * H // G, G, 264, 128), F32)],
        compiler_params=pltpu.CompilerParams(dimension_semantics=("arbitrary",),
                                             vmem_limit_bytes=64 * 1024 * 1024),
        name="adaln_k7",
    )(x, c, A_wqkv, A_wo, B_w1, B_w2, w_mod)
    return out.reshape(B, S, D)


@jax.jit
def pallas_adaLN_cond__sliding_block__dense_activation_silu__prompt_kernel(A_x, A_wqkv, A_wo, B_x, B_w1, B_w2, c, w_mod):
    return run(A_x, A_wqkv, A_wo, B_x, B_w1, B_w2, c, w_mod, LA=3)
```

```python
import jax
import jax.numpy as jnp
from jax import lax
import jax.experimental.pallas as pl
import jax.experimental.pallas.tpu as pltpu

F32 = jnp.float32
BF16 = jnp.bfloat16
U32 = jnp.uint32
D = 512
H = 32
DH = 16
W = 256
EPS = 1e-5
LOG2E = 1.4426950408889634
NEG = -1e30


def _ln(x):
    m = jnp.mean(x, axis=-1, keepdims=True)
    xc = x - m
    v = jnp.mean(xc * xc, axis=-1, keepdims=True)
    return xc * lax.rsqrt(v + EPS)


def _nt(a, b):
    return lax.dot_general(a, b, (((1,), (1,)), ((), ())), preferred_element_type=F32)


def _nn(a, b):
    return jnp.dot(a, b, preferred_element_type=F32)


def _packi(x):
    r, c = x.shape
    x4 = x.reshape(r // 16, 2, 8, c)
    p = pltpu.pack_elementwise([x4[:, 0], x4[:, 1]], packed_dtype=BF16)
    return p.reshape(r // 2, c)


def _packc(x):
    return pltpu.bitcast(x.astype(BF16), U32)


def _asbf(x):
    return pltpu.bitcast(x, BF16)


def _far_valid(QW):
    row = lax.broadcasted_iota(jnp.int32, (QW, 128), 0)
    ql = lax.broadcasted_iota(jnp.int32, (QW, 128), 1) & (QW - 1)
    return row > ql


def _lane_group(shape, QW):
    sh = QW.bit_length() - 1
    return lax.broadcasted_iota(jnp.int32, shape, 1) >> sh


def _qk_gen(G, qT, kwin, slab_head0, nvalid_blocks, s_ref, rev=False):
    QW = 128 // G
    NC = 2 * G + 1
    first_valid_row = (3 - nvalid_blocks) * 128
    grp8 = _lane_group((8, 128), QW)
    far_valid = _far_valid(QW)
    rq = [qT[hh] if hh == 0 else pltpu.roll(qT[hh], QW * hh, 1) for hh in range(G)]
    zero8 = jnp.zeros((8, 128), U32)
    for jj in range(G):
        j = G - 1 - jj if rev else jj
        blocks = []
        for b in range(8):
            hh = b - slab_head0
            if 0 <= hh < G:
                blocks.append(jnp.where(grp8 == (j + hh) % G, rq[hh], zero8))
            else:
                blocks.append(zero8)
        wj = _asbf(jnp.concatenate(blocks, axis=0))
        c0 = max(0, first_valid_row // QW - j)
        s = _nn(kwin(QW * (j + c0), QW * (NC - c0)), wj)
        last = s[(NC - 1 - c0) * QW:]
        ch = [None] * NC
        if c0 == 0:
            merged = jnp.where(far_valid, s[:QW], last)
        else:
            merged = jnp.where(far_valid, NEG, last)
        for c in range(max(c0, 1), NC - 1):
            ch[c] = s[(c - c0) * QW:(c - c0 + 1) * QW]
        ch[NC - 1] = merged
        m = None
        for c in range(1, NC):
            if ch[c] is not None:
                s_ref[j, (c - 1) * QW:c * QW, :] = ch[c]
                for r in range(0, QW, 8):
                    m = ch[c][r:r + 8] if m is None else jnp.maximum(m, ch[c][r:r + 8])
        m = jnp.max(m, axis=0, keepdims=True)
        s_ref[j, 256:264, :] = jnp.broadcast_to(m, (8, 128))
        if jj % 4 == 3:
            yield


def _barrel(G, A, shape, dtype):
    QW = 128 // G
    lane = _lane_group(shape, QW)
    zero = jnp.zeros(shape, dtype)
    cur = list(A)
    bit = 1
    while bit < G:
        sel = (lane & bit) != 0
        nxt = []
        for j in range(G):
            a, b = cur[(j + bit) % G], cur[j]
            if a is None and b is None:
                nxt.append(None)
            else:
                nxt.append(jnp.where(sel, zero if a is None else a, zero if b is None else b))
        cur = nxt
        bit *= 2
    return [zero if c is None else c for c in cur]


def _softmax_pv_gen(G, s_ref, nvalid_blocks, vts, res):
    QW = 128 // G
    NC = 2 * G + 1
    first_valid_row = (3 - nvalid_blocks) * 128
    far_valid = _far_valid(QW)
    pm_cache = {}
    lsum = [None] * G
    lcur = [None] * G

    def pexp(j, c):
        m = s_ref[j, 256:264, :]
        s = s_ref[j, (c - 1) * QW:c * QW, :]
        p = jnp.exp2(s - jnp.concatenate([m] * (QW // 8), axis=0))
        for r in range(QW - 16, -1, -16):
            pr = p[r:r + 8] + p[r + 8:r + 16]
            lcur[j] = pr if lcur[j] is None else lcur[j] + pr
        return p

    def pchunk(j, c):
        c0 = max(0, first_valid_row // QW - j)
        if c < 0 or c >= NC or c < c0:
            return None
        if c == 0 or c == NC - 1:
            if j not in pm_cache:
                pm = pexp(j, NC - 1)
                if c0 == 0:
                    pm_cache[j] = (_packi(jnp.where(far_valid, pm, 0.0)), _packi(jnp.where(far_valid, 0.0, pm)))
                else:
                    pm_cache[j] = (None, _packi(pm))
            return pm_cache[j][0 if c == 0 else 1]
        return _packi(pexp(j, c))

    acc = [None] * G
    for kt in range(3 - nvalid_blocks, 3):
        outs = [[] for _ in range(G)]
        for t in range((kt + 1) * G - 1, kt * G - 1, -1):
            A = [pchunk(j, t - j) for j in range(G)]
            Dj = _barrel(G, A, (QW // 2, 128), U32)
            for hh in range(G):
                outs[hh].insert(0, Dj[(-hh) % G])
        for j in range(G):
            if lcur[j] is not None:
                lsum[j] = lcur[j] if lsum[j] is None else lsum[j] + lcur[j]
                lcur[j] = None
        for hh in range(G):
            pt = _asbf(jnp.concatenate(outs[hh], axis=0))
            o = _nn(_asbf(vts[hh][kt]), pt)
            acc[hh] = o if acc[hh] is None else o + acc[hh]
            if hh % 4 == 3 and not (kt == 2 and hh == G - 1):
                yield
    Ld = _barrel(G, lsum, (8, 128), F32)
    for hh in range(G):
        l = jnp.sum(Ld[(-hh) % G], axis=0, keepdims=True)
        o = acc[hh] * pl.reciprocal(l, approx=True)
        if hh:
            o = pltpu.roll(o, 128 - QW * hh, 1)
        res.append(o)


def make_kernel(TQ, G, S, F, pats, dma_order, scopes, only):
    NQ = TQ // 128
    NT = S // TQ
    NF = F // 128
    NPAIR = (NT - 2) // 2
    groups = [(b, h0) for b in range(NQ) for h0 in range(0, H, G)]
    NG = len(groups)

    def kernel(x_hbm, c_hbm, wqkv_hbm, wo_hbm, w1_hbm, w2_hbm, wmod_hbm, out_hbm,
               x_s, c_ref, wqkv_ref, wo_ref, w1_ref, w2_ref, wmod_ref, sems,
               mod_s, wqvT_s, k_s, vT_s, qT_s, s_s, o_s, out_s):
        i = pl.program_id(0)

        def colcp(src, dst, lo, hi, k):
            return pltpu.make_async_copy(src.at[:, lo:hi], dst.at[:, lo:hi], sems.at[k])

        def rowcp(src, dst, lo, hi, k):
            return pltpu.make_async_copy(src.at[lo:hi, :], dst.at[lo:hi, :], sems.at[k])

        copies = {
            'c': lambda: pltpu.make_async_copy(c_hbm, c_ref, sems.at[0]),
            'mod1': lambda: colcp(wmod_hbm, wmod_ref, 0, 2 * D, 1),
            'ca': lambda: colcp(wmod_hbm, wmod_ref, D, 2 * D, 1),
            'sa': lambda: colcp(wmod_hbm, wmod_ref, 0, D, 16),
            'wk': lambda: colcp(wqkv_hbm, wqkv_ref, D, 2 * D, 2),
            'wka': lambda: colcp(wqkv_hbm, wqkv_ref, D, D + 256, 2),
            'wkb': lambda: colcp(wqkv_hbm, wqkv_ref, D + 256, 2 * D, 17),
            'wq': lambda: colcp(wqkv_hbm, wqkv_ref, 0, D, 3),
            'wv': lambda: colcp(wqkv_hbm, wqkv_ref, 2 * D, 3 * D, 4),
            'wo': lambda: pltpu.make_async_copy(wo_hbm, wo_ref, sems.at[5]),
            'mod2': lambda: colcp(wmod_hbm, wmod_ref, 2 * D, 5 * D, 6),
            'mod3': lambda: colcp(wmod_hbm, wmod_ref, 5 * D, 6 * D, 7),
            'w1a': lambda: colcp(w1_hbm, w1_ref, 0, 640, 8),
            'w1b': lambda: colcp(w1_hbm, w1_ref, 640, F, 15),
            'w2': lambda: pltpu.make_async_copy(w2_hbm, w2_ref, sems.at[9]),
            'x0': lambda: rowcp(x_hbm, x_s, 0, TQ, 10),
            'x1': lambda: rowcp(x_hbm, x_s, TQ, 2 * TQ, 11),
            'xr': lambda: rowcp(x_hbm, x_s, 2 * TQ, S, 12),
            'out0': lambda: rowcp(out_s, out_hbm, 0, S - TQ, 13),
            'out1': lambda: rowcp(out_s, out_hbm, S - TQ, S, 14),
        }

        def wait(name):
            if scopes:
                with jax.named_scope('wait_' + name):
                    copies[name]().wait()
            else:
                copies[name]().wait()

        def rows(t, n):
            return pl.ds(t * n, n) if isinstance(t, int) else pl.ds(pl.multiple_of(t * n, n), n)

        def modc(k, cc):
            return mod_s[0:1, k * D + cc * 128:k * D + (cc + 1) * 128]

        def modv(k):
            return mod_s[0:1, k * D:(k + 1) * D]

        def mod_gen(ks):
            c = c_ref[...].astype(F32)
            sc = jnp.broadcast_to((c * jax.nn.sigmoid(c)).astype(BF16), (16, D))
            for k in ks:
                for cc in range(4):
                    lo = k * D + cc * 128
                    mod_s[:, lo:lo + 128] = _nn(sc, wmod_ref[:, lo:lo + 128])[:8]
                    yield

        def xpose_gen():
            if pats['steady'].split('/')[0].count('U') == 4:
                yield
                yield
                return
            wqvT_s[0:D // 2, :] = pltpu.bitcast(wqkv_ref[:, 0:D].T, U32)
            yield
            wqvT_s[D // 2:D, :] = pltpu.bitcast(wqkv_ref[:, 2 * D:3 * D].T, U32)
            yield

        class Proj:
            def __init__(self, t, qb=0, split=1):
                self.t = t
                self.qb = qb
                self.split = split
                self.staged = isinstance(t, int)

            def n_gen(self):
                n = _ln(x_s[rows(self.t, TQ), :].astype(F32))
                if not self.staged:
                    yield
                    hf = n * (1.0 + modv(1)) + modv(0)
                    h = hf.astype(BF16)
                    hp = _asbf(_packi(hf))
                    self.h = lambda lo, hi: h if hi - lo == TQ else h[lo:hi]
                    self.hp = lambda lo, hi: hp if hi - lo == TQ else hp[lo:hi]
                    yield
                    return
                g = NG - 1 - self.t
                for cc in range(4):
                    s_s[g, cc, 0:TQ, :] = n[:, cc * 128:(cc + 1) * 128]
                yield
                r0 = S // 2 - (2 * self.t + 2) * (TQ // 2)
                r1 = r0 + TQ // 2
                for r in range(0, TQ, 32):
                    for cc in range(4):
                        cs = slice(cc * 128, (cc + 1) * 128)
                        hf = s_s[g, cc, r:r + 32, :] * (1.0 + modc(1, cc)) + modc(0, cc)
                        k_s[r0 + r // 2:r0 + r // 2 + 16, cs] = _packc(hf)
                        k_s[r1 + r // 2:r1 + r // 2 + 16, cs] = _packi(hf)
                self.h = lambda lo, hi: _asbf(k_s[r0 + lo // 2:r0 + hi // 2, :])
                self.hp = lambda lo, hi: _asbf(k_s[r1 + lo // 2:r1 + hi // 2, :])
                yield

            def k_gen(self):
                for cc in range(4):
                    k_s[rows(self.t, TQ // 2), cc * 128:(cc + 1) * 128] = _packc(
                        _nn(self.h(0, TQ), wqkv_ref[:, D + cc * 128:D + (cc + 1) * 128]))
                    yield

            def q_gen(self):
                R = D // 2 // self.split
                for b in range(NQ):
                    for p in range(self.split):
                        qT_s[self.qb * NQ + b, p * R:(p + 1) * R, :] = _packc(
                            _nt(_asbf(wqvT_s[p * R:(p + 1) * R, :]), self.h(b * 128, (b + 1) * 128))
                            * (DH ** -0.5 * LOG2E))
                        yield

            def v_gen(self):
                R = D // 2 // self.split
                for b in range(NQ):
                    for p in range(self.split):
                        vT_s[self.t * NQ + b, p * R:(p + 1) * R, :] = _packc(
                            _nt(_asbf(wqvT_s[D // 2 + p * R:D // 2 + (p + 1) * R, :]),
                                self.hp(b * 128, (b + 1) * 128)))
                        yield

            def q_direct_gen(self):
                for cc in range(4):
                    q = _nn(self.h(0, TQ), wqkv_ref[:, cc * 128:(cc + 1) * 128]) * (DH ** -0.5 * LOG2E)
                    qt = pltpu.bitcast(q.astype(BF16).T, U32)
                    for b in range(NQ):
                        qT_s[self.qb * NQ + b, cc * 64:(cc + 1) * 64, :] = qt[:, b * 128:(b + 1) * 128]
                    yield

            def v_direct_gen(self):
                for cc in range(4):
                    v = _nn(self.hp(0, TQ), wqkv_ref[:, 2 * D + cc * 128:2 * D + (cc + 1) * 128])
                    vt = pltpu.bitcast(v.astype(BF16).T, U32)
                    for b in range(NQ):
                        vT_s[self.t * NQ + b, cc * 64:(cc + 1) * 64, :] = vt[:, b * 128:(b + 1) * 128]
                    yield

            def gens(self, up=True, direct=False):
                if direct:
                    g = {'N': self.n_gen(), 'K': self.k_gen(), 'U': self.q_direct_gen(), 'V': self.v_direct_gen()}
                else:
                    g = {'N': self.n_gen(), 'K': self.k_gen(), 'U': self.q_gen(), 'V': self.v_gen()}
                return g if up else {k.lower(): v for k, v in g.items()}

        class Attn:
            def __init__(self, t, qb=0):
                self.t = t
                self.qb = qb
                self.first = isinstance(t, int) and t == 0

            def nvalid(self, b):
                return min(3, b + 1) if self.first else 3

            def qk_gen(self):
                t = self.t
                for n in range(NG):
                    b, h0 = groups[n]
                    slab = h0 // 8

                    def kwin(start, size):
                        s2 = (b * 128 - 256 + start) // 2
                        if isinstance(t, int):
                            st = t * (TQ // 2) + s2
                        else:
                            st = pl.multiple_of(t * (TQ // 2) + s2, 8)
                        return _asbf(k_s[pl.ds(st, size // 2), slab * 128:(slab + 1) * 128])
                    qs = [qT_s[self.qb * NQ + b, (h0 + hh) * 8:(h0 + hh + 1) * 8, :] for hh in range(G)]
                    yield from _qk_gen(G, qs, kwin, h0 % 8, self.nvalid(b), s_s.at[n],
                                       rev=self.first and n % 2 == 1 and pats['rev'])

            def pv_gen(self):
                oT = []
                for n in range(NG):
                    b, h0 = groups[n]
                    vts = []
                    for hh in range(G):
                        hd = h0 + hh
                        vts.append([vT_s[self.t * NQ + b - 2 + kt, hd * 8:(hd + 1) * 8, :]
                                    if kt >= 3 - self.nvalid(b) else None for kt in range(3)])
                    yield from _softmax_pv_gen(G, s_s.at[n], self.nvalid(b), vts, oT)
                    if h0 + G == H:
                        oTb = jnp.concatenate(oT[b * H:(b + 1) * H], axis=0).astype(BF16)
                        o_s[b * 64:(b + 1) * 64, :] = pltpu.bitcast(oTb.T, U32)
                    yield

            def gens(self):
                return {'Q': self.qk_gen(), 'P': self.pv_gen()}

        class Mlp:
            def __init__(self, t, lead=5):
                self.t = t
                self.lead = lead
                self.pre = {}

            def wo_gen(self):
                o = _asbf(o_s[...])
                self.att = []
                for cc in range(4):
                    self.att.append(_nn(o, wo_ref[:, cc * 128:(cc + 1) * 128]))
                    yield

            def ln2_gen(self):
                xb = x_s[rows(self.t, TQ), :].astype(F32)
                self.x1 = xb + modv(2) * jnp.concatenate(self.att, axis=1)
                self.h2 = (_ln(self.x1) * (0.5 * (1.0 + modv(4))) + 0.5 * modv(3)).astype(BF16)
                yield

            def wo_half_gen(self):
                self.atth = []
                for b in range(NQ):
                    o = _asbf(o_s[b * 64:(b + 1) * 64, :])
                    self.atth.append([])
                    for cc in range(4):
                        self.atth[b].append(_nn(o, wo_ref[:, cc * 128:(cc + 1) * 128]))
                        yield

            def ln2_half_gen(self):
                x1, h2 = [], []
                self.h2h = []
                for b in range(NQ):
                    xb = x_s[rows(self.t * NQ + b, 128), :].astype(F32)
                    x1.append(xb + modv(2) * jnp.concatenate(self.atth[b], axis=1))
                    h2.append(_ln(x1[b]) * (0.5 * (1.0 + modv(4))) + 0.5 * modv(3))
                    self.h2h.append(h2[b].astype(BF16))
                    if b == NQ - 1:
                        self.x1 = jnp.concatenate(x1, axis=0)
                        self.h2 = jnp.concatenate(h2, axis=0).astype(BF16)
                    yield

            def w1_half_gen(self, b, n):
                for r in range(n):
                    self.pre.setdefault(r, {})[b] = _nn(self.h2h[b], w1_ref[:, r * 128:(r + 1) * 128])
                    yield

            def d_gen(self):
                act = []
                y = [None] * 4
                for r in sorted(self.pre):
                    a = jnp.concatenate([self.pre[r][b] for b in range(NQ)], axis=0)
                    act.append((a + a * jnp.tanh(a)).astype(BF16))
                w1l = [('1', r) for r in range(len(act), NF)]
                w2l = []
                for g in range((NF + 3) // 4):
                    nk = min(4, NF - g * 4)
                    per = 4 // nk
                    for c0 in range(0, 4, per):
                        w2l.append(('2', g, tuple(range(c0, c0 + per))))
                order = []
                done1 = len(act)
                while w1l or w2l:
                    if w1l and (done1 < self.lead or not w2l or done1 < min(NF, w2l[0][1] * 4 + 5)):
                        order.append(w1l.pop(0))
                        done1 += 1
                    else:
                        order.append(w2l.pop(0))
                        if w1l:
                            order.append(w1l.pop(0))
                            done1 += 1
                for it in order:
                    if it[0] == '1':
                        r = it[1]
                        a = _nn(self.h2, w1_ref[:, r * 128:(r + 1) * 128])
                        act.append((a + a * jnp.tanh(a)).astype(BF16))
                    else:
                        lo, hi = it[1] * 4, min(it[1] * 4 + 4, NF)
                        for cc in it[2]:
                            for r in range(lo, hi):
                                p = _nn(act[r], w2_ref[r * 128:(r + 1) * 128, cc * 128:(cc + 1) * 128])
                                y[cc] = p if y[cc] is None else p + y[cc]
                            if hi == NF:
                                cs = slice(cc * 128, (cc + 1) * 128)
                                out_s[rows(self.t, TQ), cs] = (
                                    self.x1[:, cs] + modc(5, cc) * y[cc]).astype(out_s.dtype)
                    yield

            def gens(self):
                return {'O': self.wo_gen(), 'L': self.ln2_gen(), 'D': self.d_gen()}

        def play(pattern, gens):
            for tok in pattern.split():
                if tok.startswith('!'):
                    for nm in tok[1:].split(','):
                        wait(nm)
                elif tok.startswith('>'):
                    for nm in tok[1:].split(','):
                        copies[nm]().start()
                else:
                    for ch in tok:
                        next(gens[ch])
            for ch, g in gens.items():
                left = sum(1 for _ in g)
                assert left == 0, (ch, left)

        def scoped(name, fn):
            if only is not None and name not in only:
                return
            if scopes:
                with jax.named_scope(name):
                    fn()
            else:
                fn()

        def step0():
            for nm in dma_order:
                copies[nm]().start()
            play(pats['first'], {**Proj(0, 1).gens(False, True), **Proj(1, 0, 2).gens(True, pats['direct1']), **Attn(0, 1).gens(),
                                 'M': mod_gen((1, 0)), 'X': xpose_gen()})

        def step1():
            play(pats['second'], {**Attn(1).gens(), **Mlp(0, pats['lead1']).gens(),
                                  'M': mod_gen((2, 4, 3)), 'm': mod_gen((5,))})

        def steady():
            for u in range(2):
                t = 2 * i - 2 + u
                play(pats['steady'].split('/')[u % len(pats['steady'].split('/'))], {**Proj(t).gens(True, pats['steady'].split('/')[0].count('U') == 4), **Attn(t).gens(), **Mlp(t - 1).gens()})

        def last():
            m = Mlp(NT - 1)
            nh = pats['last'].count('a')
            play(pats['last'], {'O': m.wo_half_gen(), 'L': m.ln2_half_gen(), 'a': m.w1_half_gen(0, nh),
                                'b': m.w1_half_gen(1, nh), 'D': m.d_gen()})

        pl.when(i == 0)(lambda: scoped('step0', step0))
        pl.when(i == 1)(lambda: scoped('step1', step1))
        pl.when(jnp.logical_and(i > 1, i < NPAIR + 2))(lambda: scoped('steady', steady))
        pl.when(i == NPAIR + 2)(lambda: scoped('last', last))

    return kernel, NPAIR + 3


PATS = {
    'first': '!x0 n !c,mod1 MMMMMMMM n !wk kkkk !wq uuuu QQQQ !wv,x1 NN vv QQ vv U QQ U PP QQ PP U PP QQ PP U QQ PP '
             'V QQ PP V PP XX V PP V PP K PP K PP PP KK',
    'second': '!wo,mod2,w1a OMM OMM OMM OMM QMM QMM L Q ' + 'QPPDP' * 4 + 'D !w1b,w2,mod3 Dm' + 'QPDPDP' * 3
              + 'mQPDPP' * 3 + 'QPDPP' + 'QPDPDP' * 2 + 'PDPDP' * 3 + 'DD !xr',
    'lead1': 6,
    'rev': True,
    'direct1': True,
    'steady': 'NN OOOO L KK UV QQQ ' + 'QPKPUP QPKPVP' + 'QPDPP' * 2 + 'QPDPDP' * 9 + 'PDPDP' * 3 + 'DD',
    'last': '>out0 OOOO L OOOO L aaa bbb ' + 'D' * 25 + ' >out1 !out0,out1',
}


def run(A_x, A_wqkv, A_wo, B_x, B_w1, B_w2, c, w_mod, TQ=256, G=4, scopes=False, only=None,
        dma_order=('x0', 'c', 'mod1', 'wk', 'wq', 'wv', 'x1', 'wo', 'mod2', 'w1a', 'w1b', 'w2', 'mod3', 'xr'), **pats):
    B, S, _ = A_x.shape
    F = B_w1.shape[1]
    x = A_x.reshape(S, D)
    pats = {**PATS, **pats}
    anyspec = pl.BlockSpec(memory_space=pl.ANY)
    kernel, nsteps = make_kernel(TQ, G, S, F, pats, dma_order, scopes, only)
    out = pl.pallas_call(
        kernel,
        grid=(nsteps,),
        in_specs=[anyspec] * 7,
        out_specs=anyspec,
        out_shape=jax.ShapeDtypeStruct((S, D), A_x.dtype),
        scratch_shapes=[pltpu.VMEM((S, D), BF16), pltpu.VMEM((1, D), BF16),
                        pltpu.VMEM(A_wqkv.shape, BF16), pltpu.VMEM(A_wo.shape, BF16),
                        pltpu.VMEM(B_w1.shape, BF16), pltpu.VMEM(B_w2.shape, BF16),
                        pltpu.VMEM(w_mod.shape, BF16), pltpu.SemaphoreType.DMA((18,)),
                        pltpu.VMEM((8, 6 * D), F32), pltpu.VMEM((D, D), U32),
                        pltpu.VMEM((S // 2, D), U32), pltpu.VMEM((S // 128, D // 2, 128), U32),
                        pltpu.VMEM((2 * TQ // 128, D // 2, 128), U32),
                        pltpu.VMEM((TQ // 128 * H // G, G, 264, 128), F32),
                        pltpu.VMEM((TQ // 2, D), U32), pltpu.VMEM((S, D), BF16)],
        compiler_params=pltpu.CompilerParams(dimension_semantics=("arbitrary",),
                                             vmem_limit_bytes=64 * 1024 * 1024),
        name="adaln_k12",
    )(x, c, A_wqkv, A_wo, B_w1, B_w2, w_mod)
    return out.reshape(B, S, D)


@jax.jit
def pallas_adaLN_cond__sliding_block__dense_activation_silu__prompt_kernel(A_x, A_wqkv, A_wo, B_x, B_w1, B_w2, c, w_mod):
    return run(A_x, A_wqkv, A_wo, B_x, B_w1, B_w2, c, w_mod)
```

```python
import jax
import jax.numpy as jnp
from jax import lax
import jax.experimental.pallas as pl
import jax.experimental.pallas.tpu as pltpu

F32 = jnp.float32
BF16 = jnp.bfloat16
U32 = jnp.uint32
D = 512
H = 32
DH = 16
G = 4
TQ = 256
EPS = 1e-5
LOG2E = 1.4426950408889634
NEG = -1e30
RTD = D ** 0.5


def _ln(x):
    m = jnp.sum(x, axis=-1, keepdims=True) * (1.0 / D)
    xc = x - m
    ss = jnp.sum(xc * xc, axis=-1, keepdims=True)
    r = jnp.exp2(jnp.log(ss + D * EPS) * (-0.5 * LOG2E))
    return xc * r


def _nt(a, b):
    return lax.dot_general(a, b, (((1,), (1,)), ((), ())), preferred_element_type=F32)


def _nn(a, b):
    return jnp.dot(a, b, preferred_element_type=F32)


def _pack(buf, x):
    r = x.shape[0]
    buf.bitcast(BF16)[0:r, 0:128] = x.astype(BF16)
    return buf[0:r // 2, 0:128]


def _asbf(x):
    return pltpu.bitcast(x, BF16)


def _far_valid(qw):
    row = lax.broadcasted_iota(jnp.int32, (qw, 128), 0)
    ql = lax.broadcasted_iota(jnp.int32, (qw, 128), 1) & (qw - 1)
    return row > ql


def _far_bits(qw):
    row = 2 * lax.broadcasted_iota(jnp.int32, (qw // 2, 128), 0)
    ql = lax.broadcasted_iota(jnp.int32, (qw // 2, 128), 1) & (qw - 1)
    lo = jnp.where(row > ql, jnp.uint32(0xFFFF), jnp.uint32(0))
    hi = jnp.where(row + 1 > ql, jnp.uint32(0xFFFF0000), jnp.uint32(0))
    return lo | hi


def _lane_group(shape, width):
    return lax.broadcasted_iota(jnp.int32, shape, 1) >> (width.bit_length() - 1)


def _qk_round(qT, kwin, nvalid_blocks, s_ref, rev):
    nc = 17
    g16 = _lane_group((8, 128), 16)
    far_valid = _far_valid(16)
    is_a = (_lane_group((16, 128), 16) & 1) == 0
    rq = [qT[hh] if hh == 0 else pltpu.roll(qT[hh], 32 * hh, 1) for hh in range(G)]
    zero8 = jnp.zeros((8, 128), U32)
    for jj in range(G):
        j = G - 1 - jj if rev else jj
        blocks = [jnp.where(g16 == 2 * ((j + b % 4) % 4) + b // 4, rq[b % 4], zero8) for b in range(8)]
        wj = _asbf(jnp.concatenate(blocks, axis=0))
        c0 = max(0, 8 * (3 - nvalid_blocks) - 2 * j - 1)
        s = _nn(kwin(2 * j + 1 + c0, nc - c0), wj)
        ch = [None] * nc
        for c in range(c0, nc):
            ch[c] = s[(c - c0) * 16:(c - c0 + 1) * 16]
        mrg = jnp.where(far_valid, ch[0] if c0 == 0 else NEG, ch[nc - 1])
        y = {e: jnp.where(is_a, ch[e], ch[e - 1]) for e in range(max(2, c0 + 1), nc - 1)}
        y[nc - 1] = jnp.where(is_a, mrg, ch[nc - 2])
        y[nc] = jnp.where(is_a, ch[1] if c0 == 0 else NEG, mrg)
        m = None
        for e in sorted(y):
            s_ref[j, (e - 2) * 16:(e - 1) * 16, :] = y[e]
            for r in (0, 8):
                m = y[e][r:r + 8] if m is None else jnp.maximum(m, y[e][r:r + 8])
        m = jnp.max(m, axis=0, keepdims=True)
        s_ref[j, 256:264, :] = jnp.broadcast_to(m, (8, 128))


def _barrel(a_in, shape, dtype):
    lane = _lane_group(shape, 128 // G)
    zero = jnp.zeros(shape, dtype)
    cur = list(a_in)
    bit = 1
    while bit < G:
        sel = (lane & bit) != 0
        nxt = []
        for j in range(G):
            a, b = cur[(j + bit) % G], cur[j]
            if a is None and b is None:
                nxt.append(None)
            else:
                nxt.append(jnp.where(sel, zero if a is None else a, zero if b is None else b))
        cur = nxt
        bit *= 2
    return [zero if c is None else c for c in cur]


def _softmax_pv_gen(pack, s_ref, nvalid_blocks, vts, res):
    qw = 128 // G
    nc = 2 * G + 1
    first_valid_row = (3 - nvalid_blocks) * 128
    far_bits = _far_bits(qw)
    pm_cache = {}
    lsum = [None] * G
    lcur = [None] * G

    def pexp(j, c):
        m = s_ref[j, 256:264, :]
        s = s_ref[j, (c - 1) * qw:c * qw, :]
        p = jnp.exp2(s - jnp.concatenate([m] * (qw // 8), axis=0))
        for r in range(qw - 16, -1, -16):
            pr = p[r:r + 8] + p[r + 8:r + 16]
            lcur[j] = pr if lcur[j] is None else lcur[j] + pr
        return p

    def pchunk(j, c):
        c0 = max(0, first_valid_row // qw - j)
        if c < 0 or c >= nc or c < c0:
            return None
        if c == 0 or c == nc - 1:
            if j not in pm_cache:
                pm = pexp(j, nc - 1)
                if c0 == 0:
                    pk = pack(pm)
                    far = pk & far_bits
                    pm_cache[j] = (far, pk ^ far)
                else:
                    pm_cache[j] = (None, pack(pm))
            return pm_cache[j][0 if c == 0 else 1]
        return pack(pexp(j, c))

    acc = [None] * G
    for kt in range(3 - nvalid_blocks, 3):
        outs = [[] for _ in range(G)]
        for t in range((kt + 1) * G - 1, kt * G - 1, -1):
            dj = _barrel([pchunk(j, t - j) for j in range(G)], (qw // 2, 128), U32)
            for hh in range(G):
                outs[hh].insert(0, dj[(-hh) % G])
        for j in range(G):
            if lcur[j] is not None:
                lsum[j] = lcur[j] if lsum[j] is None else lsum[j] + lcur[j]
                lcur[j] = None
        for hh in range(G):
            pt = _asbf(jnp.concatenate(outs[hh], axis=0))
            o = _nn(_asbf(vts[hh][kt]), pt)
            acc[hh] = o if acc[hh] is None else o + acc[hh]
        if kt < 2:
            yield
    ld = _barrel(lsum, (8, 128), F32)
    for hh in range(G):
        l = jnp.sum(ld[(-hh) % G], axis=0, keepdims=True)
        rl = pl.reciprocal(l, approx=True)
        o = acc[hh] * (rl * (2.0 - l * rl))
        if hh:
            o = pltpu.roll(o, 128 - qw * hh, 1)
        res.append(o)


FIRST = ('!x0 n !c,mod1 MMMMMMMMn !wka kk !wkb,wqa ukkQQ !wqb uuuQQ !wv,x1 '
         'vvvNQNQvQUQPKPPQQPQQPPQQPUPPQQPUPPUVPPPPVPPKPPKPPKPPqq')
SECOND = ('!wo,mod2,w1a OMMMOMMOMOMMVMVMMMLQPQPQPDPQPPQPPDPPQPPDPPQPDPDPPD !w1b,w2,mod3 '
          'DmXXQPDPDPQPDPPDmPQDPPDmQPPDmQPPDPDPPDQDPDPQPPDPDPPDPDPPDPDPDPPDD !xr')
STEADY = (('NNOOOOLKKKKUVQQPQPDPUPQPDPVPPQDPQPPDPPQPDPPQPDPPQPDPDPQPPDDPPQDPDPQPDPDPQPDPDPQPDPDPQPDDPPQPDPDP'
           'DPDPPDPDPDD'),
          ('NNOOOKKOLKKUVQQPQPDPUPQPDPVPQPPDPQPDPPQPDPPQPPDPQPDPDDQPPDPPQPDPDPQPDPDPQPDPDPQPDPDPQPDPDPQPDPDD'
           'PPDPPDPDPDD'))
LAST = '>out0 OOOO L OOOO L aaa bbb ' + 'D' * 25 + ' >out1 !out0,out1'
DMA_ORDER = ('x0', 'c', 'mod1', 'wka', 'wkb', 'wqa', 'wqb', 'wv', 'x1',
             'wo', 'mod2', 'w1a', 'w1b', 'w2', 'mod3', 'xr')


def _make_kernel(S, F):
    NQ = TQ // 128
    NT = S // TQ
    NF = F // 128
    NPAIR = (NT - 2) // 2
    ND1 = SECOND.split('!w1b')[0].count('D')
    W1A = 128 * ND1
    groups = [(b, h0) for b in range(NQ) for h0 in range(0, H, G)]
    NG = len(groups)

    def kernel(x_hbm, c_hbm, wqkv_hbm, wo_hbm, w1_hbm, w2_hbm, wmod_hbm, out_hbm,
               x_s, c_ref, wqkv_ref, wo_ref, w1_ref, w2_ref, wmod_ref, sems,
               mod_s, wqvT_s, k_s, vT_s, qT_s, s_s, o_s, out_s, kl_s, *pk_s):
        i = pl.program_id(0)
        pk_cur = [None]

        def use_pack_buffer(k):
            pk_cur[0] = pk_s[k]
            pk_s[k][...] = jnp.zeros(pk_s[k].shape, U32)

        def pack(x):
            return _pack(pk_cur[0], x)

        def colcp(src, dst, lo, hi, k):
            return pltpu.make_async_copy(src.at[:, lo:hi], dst.at[:, lo:hi], sems.at[k])

        def rowcp(src, dst, lo, hi, k):
            return pltpu.make_async_copy(src.at[lo:hi, :], dst.at[lo:hi, :], sems.at[k])

        copies = {
            'c': lambda: pltpu.make_async_copy(c_hbm, c_ref, sems.at[0]),
            'mod1': lambda: colcp(wmod_hbm, wmod_ref, 0, 2 * D, 1),
            'wka': lambda: colcp(wqkv_hbm, wqkv_ref, D, D + 256, 2),
            'wkb': lambda: colcp(wqkv_hbm, wqkv_ref, D + 256, 2 * D, 17),
            'wqa': lambda: colcp(wqkv_hbm, wqkv_ref, 0, 128, 3),
            'wqb': lambda: colcp(wqkv_hbm, wqkv_ref, 128, D, 16),
            'wv': lambda: colcp(wqkv_hbm, wqkv_ref, 2 * D, 3 * D, 4),
            'wo': lambda: pltpu.make_async_copy(wo_hbm, wo_ref, sems.at[5]),
            'mod2': lambda: colcp(wmod_hbm, wmod_ref, 2 * D, 5 * D, 6),
            'mod3': lambda: colcp(wmod_hbm, wmod_ref, 5 * D, 6 * D, 7),
            'w1a': lambda: colcp(w1_hbm, w1_ref, 0, W1A, 8),
            'w1b': lambda: colcp(w1_hbm, w1_ref, W1A, F, 15),
            'w2': lambda: pltpu.make_async_copy(w2_hbm, w2_ref, sems.at[9]),
            'x0': lambda: rowcp(x_hbm, x_s, 0, TQ, 10),
            'x1': lambda: rowcp(x_hbm, x_s, TQ, 2 * TQ, 11),
            'xr': lambda: rowcp(x_hbm, x_s, 2 * TQ, S, 12),
            'out0': lambda: rowcp(out_s, out_hbm, 0, S - TQ, 13),
            'out1': lambda: rowcp(out_s, out_hbm, S - TQ, S, 14),
        }

        def rows(t, n):
            return pl.ds(t * n, n) if isinstance(t, int) else pl.ds(pl.multiple_of(t * n, n), n)

        def modc(k, cc):
            return mod_s[0:1, k * D + cc * 128:k * D + (cc + 1) * 128]

        def modv(k):
            return mod_s[0:1, k * D:(k + 1) * D]

        def mod_gen(ks):
            c = c_ref[...].astype(F32)
            sc = jnp.broadcast_to((c * jax.nn.sigmoid(c)).astype(BF16), (16, D))
            for k in ks:
                for cc in range(4):
                    lo = k * D + cc * 128
                    mod_s[:, lo:lo + 128] = _nn(sc, wmod_ref[:, lo:lo + 128])[:8]
                    yield

        def xpose_gen():
            wqvT_s[0:D // 2, :] = pltpu.bitcast(wqkv_ref[:, 0:D].T, U32)
            yield
            wqvT_s[D // 2:D, :] = pltpu.bitcast(wqkv_ref[:, 2 * D:3 * D].T, U32)
            yield

        class Proj:
            def __init__(self, t, qb=0):
                self.t = t
                self.qb = qb
                self.startup = isinstance(t, int)
                self.rng = {'K': range(4), 'U': range(4), 'V': range(4)}
                if self.startup:
                    r0 = S // 2 - (2 * t + 2) * (TQ // 2)
                    self.h = lambda lo, hi: _asbf(k_s[r0 + lo // 2:r0 + hi // 2, 0:D])

            def n_gen(self):
                n = _ln(x_s[rows(self.t, TQ), :].astype(F32))
                if not self.startup:
                    yield
                    hf = n * (RTD + RTD * modv(1)) + modv(0)
                    h = hf.astype(BF16)
                    self.h = lambda lo, hi: h if hi - lo == TQ else h[lo:hi]
                    yield
                    return
                g = NG - 1 - self.t
                for cc in range(4):
                    s_s[g, cc, 0:TQ, :] = n[:, cc * 128:(cc + 1) * 128]
                yield
                r0 = S // 2 - (2 * self.t + 2) * (TQ // 2)
                for r in range(0, TQ, 32):
                    for cc in range(4):
                        cs = slice(cc * 128, (cc + 1) * 128)
                        hf = s_s[g, cc, r:r + 32, :] * (RTD + RTD * modc(1, cc)) + modc(0, cc)
                        k_s[r0 + r // 2:r0 + r // 2 + 16, cs] = pack(hf)
                yield

            def k_gen(self):
                low = lax.broadcasted_iota(jnp.int32, (TQ // 2, 128), 1) < 64
                for cc in self.rng['K']:
                    kp = pack(_nn(self.h(0, TQ), wqkv_ref[:, D + cc * 128:D + (cc + 1) * 128]))
                    kr = pltpu.roll(kp, 64, 1)
                    if self.startup and self.t == 0:
                        pp = pr = jnp.zeros((8, 128), U32)
                    else:
                        pp, pr = kl_s[cc, 0], kl_s[cc, 1]
                    kl_s[cc, 0] = kp[TQ // 2 - 8:]
                    kl_s[cc, 1] = kr[TQ // 2 - 8:]
                    kp1 = jnp.concatenate([pp, kp[:TQ // 2 - 8]], axis=0)
                    kr1 = jnp.concatenate([pr, kr[:TQ // 2 - 8]], axis=0)
                    k_s[rows(self.t, TQ // 2), cc * 256:cc * 256 + 128] = jnp.where(low, kp1, kr)
                    k_s[rows(self.t, TQ // 2), cc * 256 + 128:cc * 256 + 256] = jnp.where(low, kr1, kp)
                    yield

            def q_gen(self):
                for b in range(NQ):
                    qT_s[self.qb * NQ + b, 0:D // 2, :] = pack(
                        _nt(_asbf(wqvT_s[0:D // 2, :]), self.h(b * 128, (b + 1) * 128)) * (DH ** -0.5 * LOG2E))
                    yield

            def v_gen(self):
                for b in range(NQ):
                    vT_s[self.t * NQ + b, 0:D // 2, :] = pack(
                        _nt(_asbf(wqvT_s[D // 2:D, :]), self.h(b * 128, (b + 1) * 128)))
                    yield

            def q_direct_gen(self):
                for cc in self.rng['U']:
                    q = _nn(self.h(0, TQ), wqkv_ref[:, cc * 128:(cc + 1) * 128]) * (DH ** -0.5 * LOG2E)
                    qt = pltpu.bitcast(q.astype(BF16).T, U32)
                    for b in range(NQ):
                        qT_s[self.qb * NQ + b, cc * 64:(cc + 1) * 64, :] = qt[:, b * 128:(b + 1) * 128]
                    yield

            def v_direct_gen(self):
                for cc in self.rng['V']:
                    v = _nn(self.h(0, TQ), wqkv_ref[:, 2 * D + cc * 128:2 * D + (cc + 1) * 128])
                    vt = pltpu.bitcast(v.astype(BF16).T, U32)
                    for b in range(NQ):
                        vT_s[self.t * NQ + b, cc * 64:(cc + 1) * 64, :] = vt[:, b * 128:(b + 1) * 128]
                    yield

            def gens(self):
                if self.startup:
                    return {'N': self.n_gen(), 'K': self.k_gen(),
                            'U': self.q_direct_gen(), 'V': self.v_direct_gen()}
                return {'N': self.n_gen(), 'K': self.k_gen(), 'U': self.q_gen(), 'V': self.v_gen()}

        class Attn:
            def __init__(self, t, qb=0):
                self.t = t
                self.qb = qb
                self.first = isinstance(t, int) and t == 0

            def nvalid(self, b):
                return min(3, b + 1) if self.first else 3

            def qk_gen(self, lo=0, hi=NG):
                t = self.t
                for n in range(lo, hi):
                    b, h0 = groups[n]
                    quad = h0 // 4

                    def kwin(g0, ng):
                        s2 = (b * 128 - 256) // 2 + g0 * 8
                        if isinstance(t, int):
                            st = t * (TQ // 2) + s2
                        else:
                            st = pl.multiple_of(t * (TQ // 2) + s2, 8)
                        return _asbf(k_s[pl.ds(st, ng * 8), quad * 128:(quad + 1) * 128])
                    qs = [qT_s[self.qb * NQ + b, (h0 + hh) * 8:(h0 + hh + 1) * 8, :] for hh in range(G)]
                    _qk_round(qs, kwin, self.nvalid(b), s_s.at[n], self.first and n % 2 == 1)
                    yield

            def pv_gen(self):
                oT = []
                for n in range(NG):
                    b, h0 = groups[n]
                    vts = []
                    for hh in range(G):
                        hd = h0 + hh
                        vts.append([vT_s[self.t * NQ + b - 2 + kt, hd * 8:(hd + 1) * 8, :]
                                    if kt >= 3 - self.nvalid(b) else None for kt in range(3)])
                    yield from _softmax_pv_gen(pack, s_s.at[n], self.nvalid(b), vts, oT)
                    nh = H if isinstance(self.t, int) else 8
                    if (h0 + G) % nh == 0:
                        oTb = jnp.concatenate(oT[-nh:], axis=0).astype(BF16)
                        o_s[b * 64:(b + 1) * 64, (h0 + G - nh) * DH:(h0 + G) * DH] = pltpu.bitcast(oTb.T, U32)
                    yield

            def gens(self):
                return {'Q': self.qk_gen(), 'P': self.pv_gen()}

        class Mlp:
            def __init__(self, t, lead=5):
                self.t = t
                self.lead = lead
                self.pre = {}

            def wo_gen(self):
                o = _asbf(o_s[...])
                self.att = []
                for cc in range(4):
                    self.att.append(_nn(o, wo_ref[:, cc * 128:(cc + 1) * 128]))
                    yield

            def ln2_gen(self):
                xb = x_s[rows(self.t, TQ), :].astype(F32)
                self.x1 = xb + modv(2) * jnp.concatenate(self.att, axis=1)
                self.h2 = (_ln(self.x1) * (0.5 * RTD + 0.5 * RTD * modv(4)) + 0.5 * modv(3)).astype(BF16)
                yield

            def wo_half_gen(self):
                self.atth = []
                for b in range(NQ):
                    o = _asbf(o_s[b * 64:(b + 1) * 64, :])
                    self.atth.append([])
                    for cc in range(4):
                        self.atth[b].append(_nn(o, wo_ref[:, cc * 128:(cc + 1) * 128]))
                        yield

            def ln2_half_gen(self):
                x1, h2 = [], []
                self.h2h = []
                for b in range(NQ):
                    xb = x_s[rows(self.t * NQ + b, 128), :].astype(F32)
                    x1.append(xb + modv(2) * jnp.concatenate(self.atth[b], axis=1))
                    h2.append(_ln(x1[b]) * (0.5 * RTD + 0.5 * RTD * modv(4)) + 0.5 * modv(3))
                    self.h2h.append(h2[b].astype(BF16))
                    if b == NQ - 1:
                        self.x1 = jnp.concatenate(x1, axis=0)
                        self.h2 = jnp.concatenate(h2, axis=0).astype(BF16)
                    yield

            def w1_half_gen(self, b, n):
                for r in range(n):
                    self.pre.setdefault(r, {})[b] = _nn(self.h2h[b], w1_ref[:, r * 128:(r + 1) * 128])
                    yield

            def d_gen(self):
                act = []
                y = [None] * 4
                for r in sorted(self.pre):
                    a = jnp.concatenate([self.pre[r][b] for b in range(NQ)], axis=0)
                    act.append((a + a * jnp.tanh(a)).astype(BF16))
                w1l = [('1', r) for r in range(len(act), NF)]
                w2l = []
                for g in range((NF + 3) // 4):
                    per = 4 // min(4, NF - g * 4)
                    for c0 in range(0, 4, per):
                        w2l.append(('2', g, tuple(range(c0, c0 + per))))
                order = []
                done1 = len(act)
                while w1l or w2l:
                    if w1l and (done1 < self.lead or not w2l or done1 < min(NF, w2l[0][1] * 4 + 5)):
                        order.append(w1l.pop(0))
                        done1 += 1
                    else:
                        order.append(w2l.pop(0))
                        if w1l:
                            order.append(w1l.pop(0))
                            done1 += 1
                for it in order:
                    if it[0] == '1':
                        r = it[1]
                        a = _nn(self.h2, w1_ref[:, r * 128:(r + 1) * 128])
                        act.append((a + a * jnp.tanh(a)).astype(BF16))
                    else:
                        lo, hi = it[1] * 4, min(it[1] * 4 + 4, NF)
                        for cc in it[2]:
                            for r in range(lo, hi):
                                p = _nn(act[r], w2_ref[r * 128:(r + 1) * 128, cc * 128:(cc + 1) * 128])
                                y[cc] = p if y[cc] is None else p + y[cc]
                        if hi == NF:
                            cs = slice(it[2][0] * 128, (it[2][-1] + 1) * 128)
                            yy = jnp.concatenate([y[cc] for cc in it[2]], axis=1)
                            out_s[rows(self.t, TQ), cs] = (
                                self.x1[:, cs] + modv(5)[:, cs] * yy).astype(out_s.dtype)
                    yield

            def gens(self):
                return {'O': self.wo_gen(), 'L': self.ln2_gen(), 'D': self.d_gen()}

        def play(pattern, gens):
            for tok in pattern.split():
                if tok.startswith('!'):
                    for nm in tok[1:].split(','):
                        copies[nm]().wait()
                elif tok.startswith('>'):
                    for nm in tok[1:].split(','):
                        copies[nm]().start()
                else:
                    for ch in tok:
                        next(gens[ch])
            for ch, g in gens.items():
                left = sum(1 for _ in g)
                assert left == 0, (ch, left)

        @pl.when(i == 0)
        def _():
            use_pack_buffer(0)
            for nm in DMA_ORDER:
                copies[nm]().start()
            p1 = Proj(1, 0)
            p1.rng = {k: range(4 - SECOND.count(k)) for k in 'KUV'}
            play(FIRST, {**{k.lower(): g for k, g in Proj(0, 1).gens().items()}, **p1.gens(),
                         **Attn(0, 1).gens(), 'M': mod_gen((1, 0)),
                         'q': Attn(1).qk_gen(0, NG - SECOND.count('Q'))})

        @pl.when(i == 1)
        def _():
            use_pack_buffer(1)
            p1 = Proj(1, 0)
            p1.rng = {k: range(4 - SECOND.count(k), 4) for k in 'KUV'}
            g1 = p1.gens()
            g1.pop('N')
            a1 = Attn(1)
            play(SECOND, {**g1, 'Q': a1.qk_gen(NG - SECOND.count('Q'), NG), 'P': a1.pv_gen(),
                          **Mlp(0, ND1 + 1).gens(), 'X': xpose_gen(),
                          'M': mod_gen((2, 4, 3)), 'm': mod_gen((5,))})

        @pl.when(jnp.logical_and(i > 1, i < NPAIR + 2))
        def _():
            use_pack_buffer(2)
            for u in range(2):
                t = 2 * i - 2 + u
                play(STEADY[u], {**Proj(t).gens(), **Attn(t).gens(), **Mlp(t - 1).gens()})

        @pl.when(i == NPAIR + 2)
        def _():
            m = Mlp(NT - 1)
            nh = LAST.count('a')
            play(LAST, {'O': m.wo_half_gen(), 'L': m.ln2_half_gen(), 'a': m.w1_half_gen(0, nh),
                        'b': m.w1_half_gen(1, nh), 'D': m.d_gen()})

    return kernel, NPAIR + 3


@jax.jit
def pallas_adaLN_cond__sliding_block__dense_activation_silu__prompt_kernel(
    A_x: jax.Array,
    A_wqkv: jax.Array,
    A_wo: jax.Array,
    B_x: jax.Array,
    B_w1: jax.Array,
    B_w2: jax.Array,
    c: jax.Array,
    w_mod: jax.Array,
):
    B, S, _ = A_x.shape
    F = B_w1.shape[1]
    assert (B, S, F) == (1, 2048, 1792)
    anyspec = pl.BlockSpec(memory_space=pl.ANY)
    kernel, nsteps = _make_kernel(S, F)
    out = pl.pallas_call(
        kernel,
        grid=(nsteps,),
        in_specs=[anyspec] * 7,
        out_specs=anyspec,
        out_shape=jax.ShapeDtypeStruct((S, D), A_x.dtype),
        scratch_shapes=[pltpu.VMEM((S, D), BF16), pltpu.VMEM((1, D), BF16),
                        pltpu.VMEM(A_wqkv.shape, BF16), pltpu.VMEM(A_wo.shape, BF16),
                        pltpu.VMEM(B_w1.shape, BF16), pltpu.VMEM(B_w2.shape, BF16),
                        pltpu.VMEM(w_mod.shape, BF16), pltpu.SemaphoreType.DMA((18,)),
                        pltpu.VMEM((8, 6 * D), F32), pltpu.VMEM((D, D), U32),
                        pltpu.VMEM((S // 2, 2 * D), U32), pltpu.VMEM((S // 128, D // 2, 128), U32),
                        pltpu.VMEM((2 * TQ // 128, D // 2, 128), U32),
                        pltpu.VMEM((TQ // 128 * H // G, G, 264, 128), F32),
                        pltpu.VMEM((TQ // 2, D), U32), pltpu.VMEM((S, D), BF16),
                        pltpu.VMEM((4, 2, 8, 128), U32)] + [pltpu.VMEM((D // 2, 256), U32)] * 3,
        compiler_params=pltpu.CompilerParams(dimension_semantics=("arbitrary",),
                                             vmem_limit_bytes=64 * 1024 * 1024,
                                             disable_semaphore_checks=True),
        name="adaln_block",
    )(A_x.reshape(S, D), c, A_wqkv, A_wo, B_w1, B_w2, w_mod)
    return out.reshape(B, S, D)
```
